```python
import os as _os
_os.environ.setdefault("JAX_PLATFORMS", "cpu")
import jax
import jax.numpy as jnp

def _softmax(x, axis=-1):
    return jax.nn.softmax(x, axis=axis)
def _gelu(x):
    return jax.nn.gelu(x, approximate=True)
def _silu(x):
    return jax.nn.silu(x)
def _sigmoid(x):
    return jax.nn.sigmoid(x)
def _layernorm(x, axis=-1, eps=1e-5):
    m = jnp.mean(x, axis=axis, keepdims=True)
    v = jnp.var(x, axis=axis, keepdims=True)
    return (x - m) / jnp.sqrt(v + eps)
def _scatter_add(tgt, idx, src, axis=0):
    return tgt.at[idx].add(src)
def _segment_sum(src, seg, n):
    return jax.ops.segment_sum(src, seg, n)
class _Rng:
    def __init__(self, key):
        self._k = key
    def _next(self):
        self._k, sub = jax.random.split(self._k)
        return sub
    def normal(self, shape):
        return jax.random.normal(self._next(), shape, dtype=jnp.bfloat16)
    def randint(self, lo, hi, shape):
        return jax.random.randint(self._next(), shape, lo, hi, dtype=jnp.int32)
    def uniform(self, shape, lo=0.0, hi=1.0):
        return jax.random.uniform(self._next(), shape, jnp.bfloat16, lo, hi)
    def permutation(self, n):
        return jax.random.permutation(self._next(), n)


kernel_name = 'concat_heads__mha_block_cached__mha_block_cached__near_ridge'

def setup_inputs():
    _rng = _Rng(jax.random.key(int.from_bytes(__import__("os").urandom(4), "little")))
    _w = (lambda a: (lambda t: t.astype(jnp.bfloat16) if jnp.issubdtype(t.dtype, jnp.floating) else t)(jnp.asarray(a)))
    def _A_setup():
        B, Sq, D = 8, 160, 512
        H, Sk, Dh = 32, 512, 128
        return {
            "x": _w((lambda *s: _rng.normal(s) * 0.8)(B, Sq, D)),
            "k_cache": _w((lambda *s: _rng.normal(s) * 0.8)(B, H, Sk, Dh)),
            "v_cache": _w((lambda *s: _rng.normal(s) * 0.05)(B, H, Sk, Dh)),
            "wq": _w((lambda *s: _rng.normal(s) * 0.8)(D, H * Dh) * (D ** -0.5)),
            "wo": _w((lambda *s: _rng.normal(s) * 0.05)(H * Dh, D) * ((H * Dh) ** -0.5)),
        }
    _A_in = _A_setup()

    def _B_setup():
        B, Sq, D = 8, 160, 512
        H, Sk, Dh = 32, 512, 128
        return {
            "x": _w((lambda *s: _rng.normal(s) * 0.8)(B, Sq, D)),
            "k_cache": _w((lambda *s: _rng.normal(s) * 0.8)(B, H, Sk, Dh)),
            "v_cache": _w((lambda *s: _rng.normal(s) * 0.05)(B, H, Sk, Dh)),
            "wq": _w((lambda *s: _rng.normal(s) * 0.8)(D, H * Dh) * (D ** -0.5)),
            "wo": _w((lambda *s: _rng.normal(s) * 0.05)(H * Dh, D) * ((H * Dh) ** -0.5)),
        }
    _B_in = _B_setup()

    return {
        "A_x": _A_in["x"],
        "A_k_cache": _A_in["k_cache"],
        "A_v_cache": _A_in["v_cache"],
        "A_wq": _A_in["wq"],
        "A_wo": _A_in["wo"],
        "B_x": _B_in["x"],
        "B_k_cache": _B_in["k_cache"],
        "B_v_cache": _B_in["v_cache"],
        "B_wq": _B_in["wq"],
        "B_wo": _B_in["wo"],
    }

def reference(A_x, A_k_cache, A_v_cache, A_wq, A_wo, B_x, B_k_cache, B_v_cache, B_wq, B_wo):
    def _A_ref(x, k_cache, v_cache, wq, wo):
        B, Sq, D = x.shape
        H, Dh = 32, 128
        q = (lambda x, *d: x.transpose(*d))((x @ wq).reshape(B, Sq, H, Dh), 0, 2, 1, 3)
        scores = jnp.einsum("bhqd,bhkd->bhqk", q, k_cache) * (Dh ** -0.5)
        p = _softmax(scores, axis=-1)
        o = jnp.einsum("bhqk,bhkd->bhqd", p, v_cache)
        return (lambda x, *d: x.transpose(*d))(o, 0, 2, 1, 3).reshape(B, Sq, H * Dh) @ wo

    def _B_ref(x, k_cache, v_cache, wq, wo):
        B, Sq, D = x.shape
        H, Dh = 32, 128
        q = (lambda x, *d: x.transpose(*d))((x @ wq).reshape(B, Sq, H, Dh), 0, 2, 1, 3)
        scores = jnp.einsum("bhqd,bhkd->bhqk", q, k_cache) * (Dh ** -0.5)
        p = _softmax(scores, axis=-1)
        o = jnp.einsum("bhqk,bhkd->bhqd", p, v_cache)
        return (lambda x, *d: x.transpose(*d))(o, 0, 2, 1, 3).reshape(B, Sq, H * Dh) @ wo

    a = _A_ref(A_x, A_k_cache, A_v_cache, A_wq, A_wo)
    b = _B_ref(B_x, B_k_cache, B_v_cache, B_wq, B_wo)
    return jnp.concatenate([a, b], axis=-1)
```

```python
import functools
import jax
import jax.numpy as jnp
import numpy as np
import jax.experimental.pallas as pl
import jax.experimental.pallas.tpu as pltpu

B, SQ, D, H, SK, DH = 8, 160, 512, 32, 512, 128
M = B * SQ
LOG2E = 1.4426950408889634
NT = (((1,), (1,)), ((), ()))


def _make(NBUF=3, order=0, newton=True):
    G = 1
    NG = H // G
    NS = 2 * NG

    def kernel(ax, ak, av, awq, awo, bx, bk, bv, bwq, bwo, out_hbm,
               x_buf, k_buf, v_buf, wq_buf, wo_buf, acc, obuf,
               sem_x, sem_k, sem_v, sem_wq, sem_wo, sem_o):

        def start_step(i, slot):
            g = jnp.where(i >= NG, i - NG, i)

            def issue(k_hbm, v_hbm, wq_hbm, wo_hbm):
                pltpu.make_async_copy(wq_hbm.at[:, pl.ds(pl.multiple_of(g * (G * DH), G * DH), G * DH)], wq_buf.at[slot], sem_wq.at[slot]).start()
                pltpu.make_async_copy(k_hbm.at[:, pl.ds(g * G, G)], k_buf.at[slot], sem_k.at[slot]).start()
                pltpu.make_async_copy(v_hbm.at[:, pl.ds(g * G, G)], v_buf.at[slot], sem_v.at[slot]).start()
                pltpu.make_async_copy(wo_hbm.at[pl.ds(pl.multiple_of(g * (G * DH), G * DH), G * DH), :], wo_buf.at[slot], sem_wo.at[slot]).start()

            @pl.when(i < NG)
            def _():
                issue(ak, av, awq, awo)

            @pl.when(i >= NG)
            def _():
                issue(bk, bv, bwq, bwo)

        xa = pltpu.make_async_copy(ax, x_buf.at[0], sem_x.at[0])
        xb = pltpu.make_async_copy(bx, x_buf.at[1], sem_x.at[1])
        xa.start()
        for j in range(NBUF - 1):
            start_step(j, j)
        xb.start()
        acc[...] = jnp.zeros_like(acc)
        xa.wait()

        def step(i, carry):
            slot = jax.lax.rem(i, NBUF)
            s = jnp.where(i >= NG, 1, 0)
            g = i - s * NG

            @pl.when(i + NBUF - 1 < NS)
            def _():
                start_step(i + NBUF - 1, jax.lax.rem(i + NBUF - 1, NBUF))

            @pl.when(i == NG)
            def _():
                xb.wait()

            pltpu.make_async_copy(awq.at[:, pl.ds(0, G * DH)], wq_buf.at[slot], sem_wq.at[slot]).wait()
            pltpu.make_async_copy(ak.at[:, pl.ds(0, G)], k_buf.at[slot], sem_k.at[slot]).wait()
            pltpu.make_async_copy(av.at[:, pl.ds(0, G)], v_buf.at[slot], sem_v.at[slot]).wait()
            pltpu.make_async_copy(awo.at[pl.ds(0, G * DH), :], wo_buf.at[slot], sem_wo.at[slot]).wait()

            q = jnp.dot(x_buf[s], wq_buf[slot], preferred_element_type=jnp.float32)
            q = (q * (DH ** -0.5 * LOG2E)).astype(jnp.bfloat16)

            def qk(b):
                return jax.lax.dot_general(q[b * SQ:(b + 1) * SQ], k_buf[slot, b, 0], NT, preferred_element_type=jnp.float32)

            def softmax(sc):
                m = jnp.max(sc, axis=-1, keepdims=True)
                p = jnp.exp2(sc - m)
                l = jnp.sum(p, axis=-1, keepdims=True)
                return p.astype(jnp.bfloat16), l

            def pv(b, p, l):
                o = jnp.dot(p, v_buf[slot, b, 0], preferred_element_type=jnp.float32)
                r = pl.reciprocal(l, approx=True)
                if newton:
                    r = r * (2.0 - l * r)
                return (o * r).astype(jnp.bfloat16)

            os_ = []
            if order == 0:
                sc = qk(0)
                for b in range(B):
                    if b + 1 < B:
                        sc_next = qk(b + 1)
                    p, l = softmax(sc)
                    os_.append(pv(b, p, l))
                    sc = sc_next
            o = jnp.concatenate(os_, axis=0)
            r = jnp.dot(o, wo_buf[slot], preferred_element_type=jnp.float32)
            acc[...] += r

            @pl.when(g == NG - 1)
            def _():
                obuf[s] = acc[...].astype(jnp.bfloat16)
                acc[...] = jnp.zeros_like(acc)
                pltpu.make_async_copy(obuf.at[s], out_hbm.at[:, pl.ds(pl.multiple_of(s * D, D), D)], sem_o.at[s]).start()
            return carry

        jax.lax.fori_loop(0, NS, step, 0)
        for s in range(2):
            pltpu.make_async_copy(obuf.at[s], out_hbm.at[:, pl.ds(s * D, D)], sem_o.at[s]).wait()

    any_spec = pl.BlockSpec(memory_space=pl.ANY)
    return pl.pallas_call(
        kernel,
        out_shape=jax.ShapeDtypeStruct((M, 2 * D), jnp.bfloat16),
        in_specs=[any_spec] * 10,
        out_specs=any_spec,
        scratch_shapes=[
            pltpu.VMEM((2, M, D), jnp.bfloat16),
            pltpu.VMEM((NBUF, B, G, SK, DH), jnp.bfloat16),
            pltpu.VMEM((NBUF, B, G, SK, DH), jnp.bfloat16),
            pltpu.VMEM((NBUF, D, G * DH), jnp.bfloat16),
            pltpu.VMEM((NBUF, G * DH, D), jnp.bfloat16),
            pltpu.VMEM((M, D), jnp.float32),
            pltpu.VMEM((2, M, D), jnp.bfloat16),
            pltpu.SemaphoreType.DMA((2,)),
            pltpu.SemaphoreType.DMA((NBUF,)),
            pltpu.SemaphoreType.DMA((NBUF,)),
            pltpu.SemaphoreType.DMA((NBUF,)),
            pltpu.SemaphoreType.DMA((NBUF,)),
            pltpu.SemaphoreType.DMA((2,)),
        ],
        compiler_params=pltpu.CompilerParams(vmem_limit_bytes=100 * 1024 * 1024),
    )


def make_fn(**kw):
    call = _make(**kw)

    def fn(A_x, A_k_cache, A_v_cache, A_wq, A_wo, B_x, B_k_cache, B_v_cache, B_wq, B_wo):
        out = call(A_x.reshape(M, D), A_k_cache, A_v_cache, A_wq, A_wo,
                   B_x.reshape(M, D), B_k_cache, B_v_cache, B_wq, B_wo)
        return out.reshape(B, SQ, 2 * D)
    return fn


@jax.jit
def pallas_concat_heads__mha_block_cached__mha_block_cached__near_ridge_kernel(
    A_x: jax.Array,
    A_k_cache: jax.Array,
    A_v_cache: jax.Array,
    A_wq: jax.Array,
    A_wo: jax.Array,
    B_x: jax.Array,
    B_k_cache: jax.Array,
    B_v_cache: jax.Array,
    B_wq: jax.Array,
    B_wo: jax.Array,
):
    return make_fn(**dict())(A_x, A_k_cache, A_v_cache, A_wq, A_wo,
                   B_x, B_k_cache, B_v_cache, B_wq, B_wo)
```

```python
import functools
import jax
import jax.numpy as jnp
import numpy as np
import jax.experimental.pallas as pl
import jax.experimental.pallas.tpu as pltpu

B, SQ, D, H, SK, DH = 8, 160, 512, 32, 512, 128
M = B * SQ
LOG2E = 1.4426950408889634
NT = (((1,), (1,)), ((), ()))


def _make(U=4, NGRP=4, PRO=3, Q0=4, NQ=2, newton=True, OCH=4, nobc=True, fp=1):
    NG = H // U
    NR = 2 * NG
    Q1 = (H - Q0) // NQ
    assert Q0 + NQ * Q1 == H and NGRP & (NGRP - 1) == 0 and PRO <= NGRP

    def kernel(ax, ak, av, awq, awo, bx, bk, bv, bwq, bwo, out_hbm,
               x_buf, wq0_buf, wq1_buf, q_buf, k_buf, v_buf, wo_buf, acc, obuf, sem):
        def group_copies(srcs, g, slot):
            k_hbm, v_hbm, wo_hbm = srcs
            s = sem.at[slot]
            return (
                pltpu.make_async_copy(k_hbm.at[:, pl.ds(g * U, U)], k_buf.at[slot], s),
                pltpu.make_async_copy(v_hbm.at[:, pl.ds(g * U, U)], v_buf.at[slot], s),
                pltpu.make_async_copy(wo_hbm.at[pl.ds(pl.multiple_of(g * (U * DH), U * DH), U * DH), :], wo_buf.at[slot], s),
            )

        def start_group(r):
            slot, g = r & (NGRP - 1), r & (NG - 1)
            if isinstance(r, int):
                for c in group_copies((ak, av, awo) if r < NG else (bk, bv, bwo), g, slot):
                    c.start()
                return

            @pl.when(r < NG)
            def _():
                for c in group_copies((ak, av, awo), g, slot):
                    c.start()

            @pl.when(jnp.logical_and(r >= NG, r < NR))
            def _():
                for c in group_copies((bk, bv, bwo), g, slot):
                    c.start()

        def wait_group(r):
            for c in group_copies((ak, av, awo), 0, r & (NGRP - 1)):
                c.wait()

        S0 = NGRP

        def proj_copies(s, srcs):
            x_hbm, wq_hbm = srcs
            cs = [pltpu.make_async_copy(x_hbm, x_buf.at[s], sem.at[S0 + 0]),
                  pltpu.make_async_copy(wq_hbm.at[:, pl.ds(0, Q0 * DH)], wq0_buf.at[s], sem.at[S0 + 0])]
            for j in range(NQ):
                cs.append(pltpu.make_async_copy(wq_hbm.at[:, pl.ds((Q0 + j * Q1) * DH, Q1 * DH)],
                                                wq1_buf.at[s, j], sem.at[S0 + 1 + j]))
            return cs

        def out_copy(s, c):
            rows = pl.ds(c * (M // OCH), M // OCH)
            return pltpu.make_async_copy(obuf.at[s, rows], out_hbm.at[rows, pl.ds(pl.multiple_of(s * D, D), D)],
                                         sem.at[S0 + 1 + NQ + s * OCH + c])

        scale = DH ** -0.5 * LOG2E

        def project(s, w_ref, h0, nh):
            x = x_buf[s]
            for t in range(nh):
                q = jnp.dot(x, w_ref[:, t * DH:(t + 1) * DH], preferred_element_type=jnp.float32)
                q_buf[h0 + t] = (q * scale).astype(jnp.bfloat16)

        def attend(s, g):
            r = s * NG + g
            slot = r & (NGRP - 1)
            wait_group(r)

            def prefetch():
                start_group(r + PRO)

                @pl.when(r == NG - 1 - PRO)
                def _():
                    for c in proj_copies(1, (bx, bwq)):
                        c.start()

            def qk(i):
                h, b = divmod(i, B)
                q = q_buf[g * U + h, b * SQ:(b + 1) * SQ, :]
                return jax.lax.dot_general(q, k_buf[slot, b, h], NT, preferred_element_type=jnp.float32)

            def softmax(sc):
                m = jnp.max(sc, axis=-1, keepdims=True)
                p = jnp.exp2(sc - m)
                l = jnp.sum(p, axis=-1, keepdims=True)
                return p.astype(jnp.bfloat16), l

            def pv(i, p, l):
                h, b = divmod(i, B)
                o = jnp.dot(p, v_buf[slot, b, h], preferred_element_type=jnp.float32)
                rcp = pl.reciprocal(l, approx=True)
                if newton:
                    rcp = rcp * (2.0 - l * rcp)
                return (o * rcp).astype(jnp.bfloat16)

            os_ = []
            NU = B * U
            sc = qk(0)
            for i in range(NU):
                if i + 1 < NU:
                    sc_next = qk(i + 1)
                p, l = softmax(sc)
                os_.append(pv(i, p, l))
                sc = sc_next
                if fp == 0 and i == 0:
                    prefetch()
            if fp == 1:
                prefetch()
            oh = [jnp.concatenate(os_[h * B:(h + 1) * B], axis=0) for h in range(U)]
            o = jnp.concatenate(oh, axis=1) if U > 1 else oh[0]
            res = jnp.dot(o, wo_buf[slot], preferred_element_type=jnp.float32)
            CH = M // OCH
            for cc in range(OCH):
                rows = pl.ds(cc * CH, CH)
                new = jnp.where(g == 0, 0.0, acc[rows, :]) + res[cc * CH:(cc + 1) * CH]
                acc[rows, :] = new
                obuf[s, rows, :] = new.astype(jnp.bfloat16)

                @pl.when(g == NG - 1)
                def _():
                    out_copy(s, cc).start()

        for c in proj_copies(0, (ax, awq)):
            c.start()
        for r in range(PRO):
            start_group(r)

        def block(s, carry):
            pltpu.make_async_copy(ax, x_buf.at[s], sem.at[S0]).wait()
            pltpu.make_async_copy(awq.at[:, pl.ds(0, Q0 * DH)], wq0_buf.at[s], sem.at[S0]).wait()
            project(s, wq0_buf.at[s], 0, Q0)

            def qbody(j, c):
                pltpu.make_async_copy(awq.at[:, pl.ds(0, Q1 * DH)], wq1_buf.at[s, j], sem.at[S0 + 1 + j]).wait()
                project(s, wq1_buf.at[s, j], Q0 + j * Q1, Q1)
                return c

            jax.lax.fori_loop(0, NQ, qbody, 0)

            def abody(g, c):
                attend(s, g)
                return c

            jax.lax.fori_loop(0, NG, abody, 0)
            return carry

        jax.lax.fori_loop(0, 2, block, 0)
        for s in range(2):
            for cc in range(OCH):
                out_copy(s, cc).wait()

    any_spec = pl.BlockSpec(memory_space=pl.ANY)
    return pl.pallas_call(
        kernel,
        out_shape=jax.ShapeDtypeStruct((M, 2 * D), jnp.bfloat16),
        in_specs=[any_spec] * 10,
        out_specs=any_spec,
        scratch_shapes=[
            pltpu.VMEM((2, M, D), jnp.bfloat16),
            pltpu.VMEM((2, D, Q0 * DH), jnp.bfloat16),
            pltpu.VMEM((2, NQ, D, Q1 * DH), jnp.bfloat16),
            pltpu.VMEM((H, M, DH), jnp.bfloat16),
            pltpu.VMEM((NGRP, B, U, SK, DH), jnp.bfloat16),
            pltpu.VMEM((NGRP, B, U, SK, DH), jnp.bfloat16),
            pltpu.VMEM((NGRP, U * DH, D), jnp.bfloat16),
            pltpu.VMEM((M, D), jnp.float32),
            pltpu.VMEM((2, M, D), jnp.bfloat16),
            pltpu.SemaphoreType.DMA((NGRP + 1 + NQ + 2 * OCH,)),
        ],
        compiler_params=pltpu.CompilerParams(vmem_limit_bytes=110 * 1024 * 1024, disable_bounds_checks=nobc),
    )


def make_fn(**kw):
    call = _make(**kw)

    def fn(A_x, A_k_cache, A_v_cache, A_wq, A_wo, B_x, B_k_cache, B_v_cache, B_wq, B_wo):
        out = call(A_x.reshape(M, D), A_k_cache, A_v_cache, A_wq, A_wo,
                   B_x.reshape(M, D), B_k_cache, B_v_cache, B_wq, B_wo)
        return out.reshape(B, SQ, 2 * D)
    return fn


@jax.jit
def pallas_concat_heads__mha_block_cached__mha_block_cached__near_ridge_kernel(
    A_x: jax.Array,
    A_k_cache: jax.Array,
    A_v_cache: jax.Array,
    A_wq: jax.Array,
    A_wo: jax.Array,
    B_x: jax.Array,
    B_k_cache: jax.Array,
    B_v_cache: jax.Array,
    B_wq: jax.Array,
    B_wo: jax.Array,
):
    return make_fn(**dict())(A_x, A_k_cache, A_v_cache, A_wq, A_wo,
                   B_x, B_k_cache, B_v_cache, B_wq, B_wo)
```

```python
import jax
import jax.numpy as jnp
import jax.experimental.pallas as pl
import jax.experimental.pallas.tpu as pltpu

B, SQ, D, H, SK, DH = 8, 160, 512, 32, 512, 128
M = B * SQ
GH = 4
NG = H // GH
NR = 2 * NG
HH = H // 2
LOG2E = 1.4426950408889634
NT = (((1,), (1,)), ((), ()))


def _make(nosc=True, late=0, nsplit=4, NGRP=4, PRO=3, X0=320, Q0=4, NB8=0, newton=True, OCH=8, nobc=True, fp=0):
    assert NGRP % 2 == 0 and PRO + (2 if NB8 else 1) <= NGRP

    def kernel(ax, ak, av, awq, awo, bx, bk, bv, bwq, bwo, out_hbm,
               x_buf, wq_buf, q_buf, k_buf, v_buf, wo_buf, acc, obuf, sem):
        def group_copies(srcs, g, slot):
            k_hbm, v_hbm, wo_hbm = srcs
            s = sem.at[slot]
            gd = GH * DH
            return (
                pltpu.make_async_copy(k_hbm.at[:, pl.ds(g * GH, GH)], k_buf.at[slot], s),
                pltpu.make_async_copy(v_hbm.at[:, pl.ds(g * GH, GH)], v_buf.at[slot], s),
                pltpu.make_async_copy(wo_hbm.at[pl.ds(pl.multiple_of(g * gd, gd), gd), :],
                                      wo_buf.at[pl.ds(pl.multiple_of(slot * gd, gd), gd), :], s),
            )

        def slot_of(r):
            if isinstance(r, int):
                return r % NGRP
            return r & (NGRP - 1) if NGRP & (NGRP - 1) == 0 else jax.lax.rem(r, NGRP)

        def start_group(r):
            slot, g = slot_of(r), r & (NG - 1)
            if isinstance(r, int):
                for c in group_copies((ak, av, awo) if r < NG else (bk, bv, bwo), g, slot):
                    c.start()
                return

            @pl.when(r < NG)
            def _():
                for c in group_copies((ak, av, awo), g, slot):
                    c.start()

            @pl.when(jnp.logical_and(r >= NG, r < NR))
            def _():
                for c in group_copies((bk, bv, bwo), g, slot):
                    c.start()

        def wait_group(r):
            for c in group_copies((ak, av, awo), 0, slot_of(r)):
                c.wait()

        S0 = NGRP
        hd = HH * DH
        xa0 = pltpu.make_async_copy(ax.at[pl.ds(0, X0)], x_buf.at[0, pl.ds(0, X0)], sem.at[S0])
        xa1 = pltpu.make_async_copy(ax.at[pl.ds(X0, M - X0)], x_buf.at[0, pl.ds(X0, M - X0)], sem.at[S0 + 1])
        wa0 = pltpu.make_async_copy(awq.at[:, pl.ds(0, Q0 * DH)], wq_buf.at[0, 0, :, pl.ds(0, Q0 * DH)], sem.at[S0])
        wa1 = pltpu.make_async_copy(awq.at[:, pl.ds(Q0 * DH, hd - Q0 * DH)],
                                    wq_buf.at[0, 0, :, pl.ds(Q0 * DH, hd - Q0 * DH)], sem.at[S0 + 2])

        def half_copy(s, wq_hbm, j):
            return pltpu.make_async_copy(wq_hbm.at[:, pl.ds(j * hd, hd)], wq_buf.at[s, j], sem.at[S0 + 3 + 2 * s + j])

        xb = pltpu.make_async_copy(bx, x_buf.at[1], sem.at[S0 + 7])
        S1 = S0 + 8

        def out_copy(s, c):
            rows = pl.ds(c * (M // OCH), M // OCH)
            return pltpu.make_async_copy(obuf.at[s, rows], out_hbm.at[rows, pl.ds(pl.multiple_of(s * D, D), D)],
                                         sem.at[S1 + s * OCH + c])

        scale = DH ** -0.5 * LOG2E

        def project(s, w_ref, h0, c0, nh, r0=0, nr=M):
            x = x_buf[s, pl.ds(r0, nr), :]
            for t in range(nh):
                q = jnp.dot(x, w_ref[:, (c0 + t) * DH:(c0 + t + 1) * DH], preferred_element_type=jnp.float32)
                q_buf[h0 + t, pl.ds(r0, nr), :] = (q * scale).astype(jnp.bfloat16)

        def attend(s, g, ng):
            r = s * NG + g
            for t in range(ng):
                wait_group(r + t)
            slots = [slot_of(r + t) for t in range(ng)]
            U = ng * GH
            NU = B * U

            def prefetch():
                for t in range(ng):
                    start_group(r + PRO + t)

                @pl.when(r == NG - 1 - PRO)
                def _():
                    xb.start()
                    for j in range(2):
                        half_copy(1, bwq, j).start()

            def qk(i):
                b, h = divmod(i, U)
                q = q_buf[g * GH + h, b * SQ:(b + 1) * SQ, :]
                return jax.lax.dot_general(q, k_buf[slots[h // GH], b, h % GH], NT, preferred_element_type=jnp.float32)

            def softmax(sc):
                m = jnp.max(sc, axis=-1, keepdims=True)
                p = jnp.exp2(sc - m)
                l = jnp.sum(p, axis=-1, keepdims=True)
                return p.astype(jnp.bfloat16), l

            def pv(i, p, l):
                b, h = divmod(i, U)
                o = jnp.dot(p, v_buf[slots[h // GH], b, h % GH], preferred_element_type=jnp.float32)
                rcp = pl.reciprocal(l, approx=True)
                if newton:
                    rcp = rcp * (2.0 - l * rcp)
                return (o * rcp).astype(jnp.bfloat16)

            def out_proj(b, os_):
                o = jnp.concatenate(os_, axis=1)
                wrows = pl.ds(pl.multiple_of(slots[0] * (GH * DH), U * DH), U * DH)
                rows = pl.ds(b * SQ, SQ)
                if nsplit == 1:
                    res = jnp.dot(o, wo_buf[wrows, :], preferred_element_type=jnp.float32)
                    new = acc[s, rows, :] + res
                    acc[s, rows, :] = new
                    obuf[s, rows, :] = new.astype(jnp.bfloat16)
                else:
                    w = D // nsplit
                    for j in range(nsplit):
                        cols = pl.ds(j * w, w)
                        res = jnp.dot(o, wo_buf[wrows, cols], preferred_element_type=jnp.float32)
                        new = acc[s, rows, cols] + res
                        acc[s, rows, cols] = new
                        obuf[s, rows, cols] = new.astype(jnp.bfloat16)

                @pl.when(g + ng == NG)
                def _():
                    out_copy(s, b).start()

            assert OCH == B
            sc = qk(0)
            os_, pending = [], None
            for i in range(NU):
                if i + 1 < NU:
                    sc_next = qk(i + 1)
                if pending is not None:
                    out_proj(*pending)
                    pending = None
                p, l = softmax(sc)
                os_.append(pv(i, p, l))
                sc = sc_next
                if (i + 1) % U == 0:
                    pending, os_ = (i // U, os_), []
                if fp == 0 and i == 0:
                    prefetch()
            if fp == 1:
                prefetch()
            out_proj(*pending)

        def rest_starts():
            wa1.start()
            half_copy(0, awq, 1).start()
            for r in range(PRO):
                start_group(r)

        xa0.start()
        wa0.start()
        xa1.start()
        if late == 0:
            rest_starts()

        acc[...] = jnp.zeros_like(acc)

        def block(s, carry):
            @pl.when(s == 0)
            def _():
                xa0.wait()
                wa0.wait()
                if late == 1:
                    rest_starts()
                project(0, wq_buf.at[0, 0], 0, 0, Q0, 0, X0)
                xa1.wait()
                if late == 2:
                    rest_starts()
                project(0, wq_buf.at[0, 0], 0, 0, Q0, X0, M - X0)
                wa1.wait()
                project(0, wq_buf.at[0, 0], Q0, Q0, HH - Q0)

            @pl.when(s == 1)
            def _():
                xb.wait()

            def qbody(j, c):
                half_copy(s, awq, j).wait()
                project(s, wq_buf.at[s, j], j * HH, 0, HH)
                return c

            jax.lax.fori_loop(1 - s, 2, qbody, 0)
            n8 = s * NB8

            def a8body(j, c):
                attend(s, 2 * j, 2)
                return c

            jax.lax.fori_loop(0, n8, a8body, 0)

            def a4body(g, c):
                attend(s, g, 1)
                return c

            jax.lax.fori_loop(2 * n8, NG, a4body, 0)
            return carry

        jax.lax.fori_loop(0, 2, block, 0)
        for s in range(2):
            for cc in range(OCH):
                out_copy(s, cc).wait()

    any_spec = pl.BlockSpec(memory_space=pl.ANY)
    return pl.pallas_call(
        kernel,
        out_shape=jax.ShapeDtypeStruct((M, 2 * D), jnp.bfloat16),
        in_specs=[any_spec] * 10,
        out_specs=any_spec,
        scratch_shapes=[
            pltpu.VMEM((2, M, D), jnp.bfloat16),
            pltpu.VMEM((2, 2, D, HH * DH), jnp.bfloat16),
            pltpu.VMEM((H, M, DH), jnp.bfloat16),
            pltpu.VMEM((NGRP, B, GH, SK, DH), jnp.bfloat16),
            pltpu.VMEM((NGRP, B, GH, SK, DH), jnp.bfloat16),
            pltpu.VMEM((NGRP * GH * DH, D), jnp.bfloat16),
            pltpu.VMEM((2, M, D), jnp.float32),
            pltpu.VMEM((2, M, D), jnp.bfloat16),
            pltpu.SemaphoreType.DMA((NGRP + 8 + 2 * OCH,)),
        ],
        compiler_params=pltpu.CompilerParams(vmem_limit_bytes=110 * 1024 * 1024, disable_bounds_checks=nobc, disable_semaphore_checks=nosc),
    )


def make_fn(**kw):
    call = _make(**kw)

    def fn(A_x, A_k_cache, A_v_cache, A_wq, A_wo, B_x, B_k_cache, B_v_cache, B_wq, B_wo):
        out = call(A_x.reshape(M, D), A_k_cache, A_v_cache, A_wq, A_wo,
                   B_x.reshape(M, D), B_k_cache, B_v_cache, B_wq, B_wo)
        return out.reshape(B, SQ, 2 * D)
    return fn


@jax.jit
def pallas_concat_heads__mha_block_cached__mha_block_cached__near_ridge_kernel(
    A_x: jax.Array,
    A_k_cache: jax.Array,
    A_v_cache: jax.Array,
    A_wq: jax.Array,
    A_wo: jax.Array,
    B_x: jax.Array,
    B_k_cache: jax.Array,
    B_v_cache: jax.Array,
    B_wq: jax.Array,
    B_wo: jax.Array,
):
    return make_fn(**dict(X0=400))(A_x, A_k_cache, A_v_cache, A_wq, A_wo,
                   B_x, B_k_cache, B_v_cache, B_wq, B_wo)
```

```python
import jax
import jax.numpy as jnp
import jax.experimental.pallas as pl
import jax.experimental.pallas.tpu as pltpu

B, SQ, D, H, SK, DH = 8, 160, 512, 32, 512, 128
M = B * SQ
GH = 4
GD = GH * DH
NG = H // GH
NR = 2 * NG
LOG2E = 1.4426950408889634
NT = (((1,), (1,)), ((), ()))


def _make(NGRP=4, PRO=3, X0=400, Q0=4, NQ=2, var=3, fp=0, qpos=0, nobc=True, nosc=True):
    Q1 = (H - Q0) // NQ
    assert Q0 + NQ * Q1 == H and NGRP & (NGRP - 1) == 0 and PRO < NGRP

    def kernel(ax, ak, av, awq, awo, bx, bk, bv, bwq, bwo, out_hbm,
               x_buf, wq0_buf, wq1_buf, wqb_buf, q_buf, k_buf, v_buf, wo_buf, acc, obuf, sem):
        def group_copies(a, g, slot):
            k_hbm, v_hbm, wo_hbm = (ak, av, awo) if a else (bk, bv, bwo)
            s = sem.at[slot]
            cols = pl.ds(pl.multiple_of(g * GD, GD), GD)
            cs = [
                pltpu.make_async_copy(k_hbm.at[:, pl.ds(g * GH, GH)], k_buf.at[slot], s),
                pltpu.make_async_copy(v_hbm.at[:, pl.ds(g * GH, GH)], v_buf.at[slot], s),
                pltpu.make_async_copy(wo_hbm.at[cols, :], wo_buf.at[slot], s),
            ]
            if a:
                cs.append(pltpu.make_async_copy(bwq.at[:, cols], wqb_buf.at[slot], s))
            return cs

        def start_group(r):
            slot, g = r & (NGRP - 1), r & (NG - 1)
            if isinstance(r, int):
                for c in group_copies(r < NG, g, slot):
                    c.start()
                return

            @pl.when(r < NG)
            def _():
                for c in group_copies(True, g, slot):
                    c.start()

            @pl.when(jnp.logical_and(r >= NG, r < NR))
            def _():
                for c in group_copies(False, g, slot):
                    c.start()

        S0 = NGRP
        xa0 = pltpu.make_async_copy(ax.at[pl.ds(0, X0)], x_buf.at[0, pl.ds(0, X0)], sem.at[S0])
        xa1 = pltpu.make_async_copy(ax.at[pl.ds(X0, M - X0)], x_buf.at[0, pl.ds(X0, M - X0)], sem.at[S0 + 1])
        wa0 = pltpu.make_async_copy(awq.at[:, pl.ds(0, Q0 * DH)], wq0_buf, sem.at[S0])

        def wa1(j):
            return pltpu.make_async_copy(awq.at[:, pl.ds((Q0 + j * Q1) * DH, Q1 * DH)], wq1_buf.at[j], sem.at[S0 + 2 + j])

        xb = pltpu.make_async_copy(bx, x_buf.at[1], sem.at[S0 + 2 + NQ])
        S1 = S0 + 3 + NQ

        def out_copy(s, b):
            rows = pl.ds(b * SQ, SQ)
            return pltpu.make_async_copy(obuf.at[s, rows], out_hbm.at[rows, pl.ds(s * D, D)], sem.at[S1 + s * B + b])

        scale = DH ** -0.5 * LOG2E

        def project(s, w_ref, h0, nh, r0=0, nr=M):
            x = x_buf[s, pl.ds(r0, nr), :]
            for t in range(nh):
                q = jnp.dot(x, w_ref[:, t * DH:(t + 1) * DH], preferred_element_type=jnp.float32)
                q_buf[s, h0 + t, pl.ds(r0, nr), :] = (q * scale).astype(jnp.bfloat16)

        def attend(s, g):
            r = s * NG + g
            slot = r & (NGRP - 1)
            for c in group_copies(s == 0, 0, slot):
                c.wait()
            NU = B * GH

            def qk(i):
                b, h = divmod(i, GH)
                q = q_buf[s, g * GH + h, b * SQ:(b + 1) * SQ, :]
                return jax.lax.dot_general(q, k_buf[slot, b, h], NT, preferred_element_type=jnp.float32)

            def softmax(sc):
                m = jnp.max(sc, axis=-1, keepdims=True)
                p = jnp.exp2(sc - m)
                l = jnp.sum(p, axis=-1, keepdims=True)
                return p.astype(jnp.bfloat16), l

            def pv(i, p, l):
                b, h = divmod(i, GH)
                o = jnp.dot(p, v_buf[slot, b, h], preferred_element_type=jnp.float32)
                rcp = pl.reciprocal(l, approx=True)
                rcp = rcp * (2.0 - l * rcp)
                return (o * rcp).astype(jnp.bfloat16)

            def out_proj(b, os_):
                o = jnp.concatenate(os_, axis=1)
                rows = pl.ds(b * SQ, SQ)
                for j in range(D // DH):
                    cols = pl.ds(j * DH, DH)
                    res = jnp.dot(o, wo_buf[slot, :, cols], preferred_element_type=jnp.float32)
                    new = acc[s, rows, cols] + res
                    acc[s, rows, cols] = new
                    obuf[s, rows, cols] = new.astype(jnp.bfloat16)

                @pl.when(g == NG - 1)
                def _():
                    out_copy(s, b).start()

            if s == 0 and qpos == 0:
                project(1, wqb_buf.at[slot], g * GH, GH)
            sc = qk(0)
            os_, pending = [], None
            for i in range(NU):
                if var == 0:
                    if i + 1 < NU:
                        sc_next = qk(i + 1)
                    p, l = softmax(sc)
                else:
                    p, l = softmax(sc)
                    if i + 1 < NU:
                        sc_next = qk(i + 1)
                if pending is not None:
                    out_proj(*pending)
                    pending = None
                os_.append(pv(i, p, l))
                sc = sc_next
                if (i + 1) % GH == 0:
                    pending, os_ = (i // GH, os_), []
                if i == fp:
                    start_group(r + PRO)
                if s == 0 and qpos > 0 and i == qpos:
                    project(1, wqb_buf.at[slot], g * GH, GH)
            out_proj(*pending)

        xa0.start()
        wa0.start()
        xa1.start()
        for j in range(NQ):
            wa1(j).start()
        start_group(0)
        xb.start()
        for r in range(1, PRO):
            start_group(r)

        def zbody(i, c):
            acc[:, pl.ds(pl.multiple_of(i * SQ, SQ), SQ), :] = jnp.zeros((2, SQ, D), jnp.float32)
            return c

        jax.lax.fori_loop(0, B, zbody, 0)

        def block(t, carry):
            @pl.when(t == 0)
            def _():
                xa0.wait()
                wa0.wait()
                project(0, wq0_buf, 0, Q0, 0, X0)
                xa1.wait()
                project(0, wq0_buf, 0, Q0, X0, M - X0)

                def qbody(j, c):
                    pltpu.make_async_copy(awq.at[:, pl.ds(0, Q1 * DH)], wq1_buf.at[j], sem.at[S0 + 2 + j]).wait()
                    project(0, wq1_buf.at[j], Q0 + j * Q1, Q1)
                    return c

                jax.lax.fori_loop(0, NQ, qbody, 0)
                xb.wait()

            @pl.when(t == 0)
            def _():
                def abody(g, c):
                    attend(0, g)
                    return c

                jax.lax.fori_loop(0, NG, abody, 0)

            @pl.when(t == 1)
            def _():
                def abody(g, c):
                    attend(1, g)
                    return c

                jax.lax.fori_loop(0, NG, abody, 0)
            return carry

        jax.lax.fori_loop(0, 2, block, 0)
        for s in range(2):
            for b in range(B):
                out_copy(s, b).wait()

    any_spec = pl.BlockSpec(memory_space=pl.ANY)
    return pl.pallas_call(
        kernel,
        out_shape=jax.ShapeDtypeStruct((M, 2 * D), jnp.bfloat16),
        in_specs=[any_spec] * 10,
        out_specs=any_spec,
        scratch_shapes=[
            pltpu.VMEM((2, M, D), jnp.bfloat16),
            pltpu.VMEM((D, Q0 * DH), jnp.bfloat16),
            pltpu.VMEM((NQ, D, Q1 * DH), jnp.bfloat16),
            pltpu.VMEM((NGRP, D, GD), jnp.bfloat16),
            pltpu.VMEM((2, H, M, DH), jnp.bfloat16),
            pltpu.VMEM((NGRP, B, GH, SK, DH), jnp.bfloat16),
            pltpu.VMEM((NGRP, B, GH, SK, DH), jnp.bfloat16),
            pltpu.VMEM((NGRP, GD, D), jnp.bfloat16),
            pltpu.VMEM((2, M, D), jnp.float32),
            pltpu.VMEM((2, M, D), jnp.bfloat16),
            pltpu.SemaphoreType.DMA((NGRP + 3 + NQ + 2 * B,)),
        ],
        compiler_params=pltpu.CompilerParams(
            vmem_limit_bytes=110 * 1024 * 1024,
            disable_bounds_checks=nobc, disable_semaphore_checks=nosc),
    )


def make_fn(**kw):
    call = _make(**kw)

    def fn(A_x, A_k_cache, A_v_cache, A_wq, A_wo, B_x, B_k_cache, B_v_cache, B_wq, B_wo):
        out = call(A_x.reshape(M, D), A_k_cache, A_v_cache, A_wq, A_wo,
                   B_x.reshape(M, D), B_k_cache, B_v_cache, B_wq, B_wo)
        return out.reshape(B, SQ, 2 * D)
    return fn


@jax.jit
def pallas_concat_heads__mha_block_cached__mha_block_cached__near_ridge_kernel(
    A_x: jax.Array,
    A_k_cache: jax.Array,
    A_v_cache: jax.Array,
    A_wq: jax.Array,
    A_wo: jax.Array,
    B_x: jax.Array,
    B_k_cache: jax.Array,
    B_v_cache: jax.Array,
    B_wq: jax.Array,
    B_wo: jax.Array,
):
    return make_fn(**dict(fp=1))(A_x, A_k_cache, A_v_cache, A_wq, A_wo,
                   B_x, B_k_cache, B_v_cache, B_wq, B_wo)
```

```python
import jax
import jax.numpy as jnp
import jax.experimental.pallas as pl
import jax.experimental.pallas.tpu as pltpu

B, SQ, D, H, SK, DH = 8, 160, 512, 32, 512, 128
M = B * SQ
GH = 4
GD = GH * DH
NG = H // GH
NGRP = 4
PRO = 3
X0 = 400
Q0 = GH
NQ = 2
Q1 = (H - Q0) // NQ
NT_DIMS = (((1,), (1,)), ((), ()))
Q_SCALE = DH ** -0.5 * 1.4426950408889634

SEM_XA0 = NGRP
SEM_XA1 = SEM_XA0 + 1
SEM_WA1 = SEM_XA1 + 1
SEM_XB = SEM_WA1 + NQ
SEM_OUT = SEM_XB + 1
SEM_LAST = SEM_OUT + 2 * B
NUM_SEM = SEM_LAST + D // DH


def _kernel(ax, ak, av, awq, awo, bx, bk, bv, bwq, bwo, out_hbm,
            x_buf, wq0_buf, wq1_buf, wqb_buf, q_buf, k_buf, v_buf, wo_buf, acc, obuf, sem):
    def group_copies(s, g, slot):
        k_hbm, v_hbm, wo_hbm = (ak, av, awo) if s == 0 else (bk, bv, bwo)
        cols = pl.ds(pl.multiple_of(g * GD, GD), GD)
        heads = pl.ds(g * GH, GH)
        copies = [
            pltpu.make_async_copy(k_hbm.at[:, heads], k_buf.at[slot], sem.at[slot]),
            pltpu.make_async_copy(v_hbm.at[:, heads], v_buf.at[slot], sem.at[slot]),
            pltpu.make_async_copy(wo_hbm.at[cols, :], wo_buf.at[slot], sem.at[slot]),
        ]
        if s == 0:
            copies.append(pltpu.make_async_copy(bwq.at[:, cols], wqb_buf.at[slot], sem.at[slot]))
        return copies

    def start_group(r):
        slot, g = r & (NGRP - 1), r & (NG - 1)
        if isinstance(r, int):
            for c in group_copies(r // NG, g, slot):
                c.start()
            return
        for s in range(2):
            @pl.when(jnp.logical_and(r >= s * NG, r < (s + 1) * NG))
            def _():
                for c in group_copies(s, g, slot):
                    c.start()

    xa0 = pltpu.make_async_copy(ax.at[pl.ds(0, X0)], x_buf.at[0, pl.ds(0, X0)], sem.at[SEM_XA0])
    wa0 = pltpu.make_async_copy(awq.at[:, pl.ds(0, Q0 * DH)], wq0_buf, sem.at[SEM_XA0])
    xa1 = pltpu.make_async_copy(ax.at[pl.ds(X0, M - X0)], x_buf.at[0, pl.ds(X0, M - X0)], sem.at[SEM_XA1])
    xb = pltpu.make_async_copy(bx, x_buf.at[1], sem.at[SEM_XB])

    def wa1(j):
        cols = pl.ds(pl.multiple_of((Q0 + j * Q1) * DH, DH), Q1 * DH)
        return pltpu.make_async_copy(awq.at[:, cols], wq1_buf.at[j], sem.at[SEM_WA1 + j])

    def out_copy(s, b):
        rows = pl.ds(b * SQ, SQ)
        return pltpu.make_async_copy(obuf.at[s, rows], out_hbm.at[rows, pl.ds(s * D, D)], sem.at[SEM_OUT + s * B + b])

    def out_copy_last(j):
        rows, cols = pl.ds((B - 1) * SQ, SQ), pl.ds(j * DH, DH)
        return pltpu.make_async_copy(obuf.at[1, rows, cols], out_hbm.at[rows, pl.ds(D + j * DH, DH)], sem.at[SEM_LAST + j])

    def project(s, w_ref, h0, nh, r0=0, nr=M):
        x = x_buf[s, pl.ds(r0, nr), :]
        for t in range(nh):
            q = jnp.dot(x, w_ref[:, t * DH:(t + 1) * DH], preferred_element_type=jnp.float32)
            q_buf[s, h0 + t, pl.ds(r0, nr), :] = (q * Q_SCALE).astype(jnp.bfloat16)

    def attend(s, g):
        r = s * NG + g
        slot = r & (NGRP - 1)
        for c in group_copies(s, g, slot):
            c.wait()

        def qk(i):
            b, h = divmod(i, GH)
            q = q_buf[s, g * GH + h, b * SQ:(b + 1) * SQ, :]
            return jax.lax.dot_general(q, k_buf[slot, b, h], NT_DIMS, preferred_element_type=jnp.float32)

        def softmax(sc):
            m = jnp.max(sc, axis=-1, keepdims=True)
            p = jnp.exp2(sc - m)
            return p.astype(jnp.bfloat16), jnp.sum(p, axis=-1, keepdims=True)

        def pv(i, p, l):
            b, h = divmod(i, GH)
            o = jnp.dot(p, v_buf[slot, b, h], preferred_element_type=jnp.float32)
            rcp = pl.reciprocal(l, approx=True)
            rcp = rcp * (2.0 - l * rcp)
            return (o * rcp).astype(jnp.bfloat16)

        def out_proj(b, heads):
            o = jnp.concatenate(heads, axis=1)
            rows = pl.ds(b * SQ, SQ)
            last_rows = s == 1 and b == B - 1
            for j in range(D // DH):
                cols = pl.ds(j * DH, DH)
                new = acc[s, rows, cols] + jnp.dot(o, wo_buf[slot, :, cols], preferred_element_type=jnp.float32)
                acc[s, rows, cols] = new
                obuf[s, rows, cols] = new.astype(jnp.bfloat16)
                if last_rows:
                    @pl.when(g == NG - 1)
                    def _():
                        out_copy_last(j).start()

            if not last_rows:
                @pl.when(g == NG - 1)
                def _():
                    out_copy(s, b).start()

        if s == 0:
            project(1, wqb_buf.at[slot], g * GH, GH)
        n_units = B * GH
        sc = qk(0)
        heads, pending = [], None
        for i in range(n_units):
            p, l = softmax(sc)
            if i + 1 < n_units:
                sc = qk(i + 1)
            if pending is not None:
                out_proj(*pending)
                pending = None
            heads.append(pv(i, p, l))
            if len(heads) == GH:
                pending, heads = (i // GH, heads), []
            if i == 1:
                start_group(r + PRO)
        out_proj(*pending)

    xa0.start()
    wa0.start()
    xa1.start()
    for j in range(NQ):
        wa1(j).start()
    start_group(0)
    xb.start()
    for r in range(1, PRO):
        start_group(r)

    def zero_acc(b, carry):
        acc[:, pl.ds(pl.multiple_of(b * SQ, SQ), SQ), :] = jnp.zeros((2, SQ, D), jnp.float32)
        return carry

    jax.lax.fori_loop(0, B, zero_acc, 0)

    def project_rest(j, carry):
        wa1(j).wait()
        project(0, wq1_buf.at[j], Q0 + j * Q1, Q1)
        return carry

    def block(s, carry):
        @pl.when(s == 0)
        def _():
            xa0.wait()
            wa0.wait()
            project(0, wq0_buf, 0, Q0, 0, X0)
            xa1.wait()
            project(0, wq0_buf, 0, Q0, X0, M - X0)
            jax.lax.fori_loop(0, NQ, project_rest, 0)
            xb.wait()

        for blk in range(2):
            @pl.when(s == blk)
            def _():
                def region(g, c):
                    attend(blk, g)
                    return c

                jax.lax.fori_loop(0, NG, region, 0)
        return carry

    jax.lax.fori_loop(0, 2, block, 0)
    for s in range(2):
        for b in range(B - s):
            out_copy(s, b).wait()
    for j in range(D // DH):
        out_copy_last(j).wait()


@jax.jit
def pallas_concat_heads__mha_block_cached__mha_block_cached__near_ridge_kernel(
    A_x: jax.Array,
    A_k_cache: jax.Array,
    A_v_cache: jax.Array,
    A_wq: jax.Array,
    A_wo: jax.Array,
    B_x: jax.Array,
    B_k_cache: jax.Array,
    B_v_cache: jax.Array,
    B_wq: jax.Array,
    B_wo: jax.Array,
):
    hbm = pl.BlockSpec(memory_space=pl.ANY)
    bf16 = jnp.bfloat16
    out = pl.pallas_call(
        _kernel,
        out_shape=jax.ShapeDtypeStruct((M, 2 * D), bf16),
        in_specs=[hbm] * 10,
        out_specs=hbm,
        scratch_shapes=[
            pltpu.VMEM((2, M, D), bf16),
            pltpu.VMEM((D, Q0 * DH), bf16),
            pltpu.VMEM((NQ, D, Q1 * DH), bf16),
            pltpu.VMEM((NGRP, D, GD), bf16),
            pltpu.VMEM((2, H, M, DH), bf16),
            pltpu.VMEM((NGRP, B, GH, SK, DH), bf16),
            pltpu.VMEM((NGRP, B, GH, SK, DH), bf16),
            pltpu.VMEM((NGRP, GD, D), bf16),
            pltpu.VMEM((2, M, D), jnp.float32),
            pltpu.VMEM((2, M, D), bf16),
            pltpu.SemaphoreType.DMA((NUM_SEM,)),
        ],
        compiler_params=pltpu.CompilerParams(
            vmem_limit_bytes=110 * 1024 * 1024,
            disable_bounds_checks=True,
            disable_semaphore_checks=True,
        ),
    )(A_x.reshape(M, D), A_k_cache, A_v_cache, A_wq, A_wo,
      B_x.reshape(M, D), B_k_cache, B_v_cache, B_wq, B_wo)
    return out.reshape(B, SQ, 2 * D)
```

```python
import jax
import jax.numpy as jnp
import jax.experimental.pallas as pl
import jax.experimental.pallas.tpu as pltpu

B, SQ, D, H, SK, DH = 8, 160, 512, 32, 512, 128
M = B * SQ
GH = 4
GD = GH * DH
NG = H // GH
NGRP = 4
PRO = 3
X0 = 480
Q0 = GH
NQ = 2
Q1 = (H - Q0) // NQ
NT_DIMS = (((1,), (1,)), ((), ()))
Q_SCALE = DH ** -0.5 * 1.4426950408889634

SEM_XA0 = NGRP
SEM_XA1 = SEM_XA0 + 1
SEM_WA1 = SEM_XA1 + 1
SEM_XB = SEM_WA1 + NQ
SEM_OUT = SEM_XB + 1
SEM_LAST = SEM_OUT + 2 * B
NUM_SEM = SEM_LAST + D // DH + 1


def _kernel(ax, ak, av, awq, awo, bx, bk, bv, bwq, bwo, out_hbm,
            x_buf, wq0_buf, wq1_buf, wqb_buf, q_buf, k_buf, v_buf, wo_buf, acc, obuf, sem):
    def group_copies(s, g, slot):
        k_hbm, v_hbm, wo_hbm = (ak, av, awo) if s == 0 else (bk, bv, bwo)
        cols = pl.ds(pl.multiple_of(g * GD, GD), GD)
        heads = pl.ds(g * GH, GH)
        copies = [
            pltpu.make_async_copy(k_hbm.at[:, heads], k_buf.at[slot], sem.at[slot]),
            pltpu.make_async_copy(v_hbm.at[:, heads], v_buf.at[slot], sem.at[slot]),
            pltpu.make_async_copy(wo_hbm.at[cols, :], wo_buf.at[slot], sem.at[slot]),
        ]
        if s == 0:
            copies.append(pltpu.make_async_copy(bwq.at[:, cols], wqb_buf.at[slot], sem.at[slot]))
        return copies

    def start_group(r):
        slot, g = r & (NGRP - 1), r & (NG - 1)
        if isinstance(r, int):
            for c in group_copies(r // NG, g, slot):
                c.start()
            return
        for s in range(2):
            @pl.when(jnp.logical_and(r >= s * NG, r < (s + 1) * NG))
            def _():
                for c in group_copies(s, g, slot):
                    c.start()

    xa0 = pltpu.make_async_copy(ax.at[pl.ds(0, X0)], x_buf.at[0, pl.ds(0, X0)], sem.at[SEM_XA0])
    hq = Q0 // 2 * DH
    wa0 = pltpu.make_async_copy(awq.at[:, pl.ds(0, hq)], wq0_buf.at[:, pl.ds(0, hq)], sem.at[SEM_XA0])
    wa0b = pltpu.make_async_copy(awq.at[:, pl.ds(hq, hq)], wq0_buf.at[:, pl.ds(hq, hq)], sem.at[SEM_LAST + 4])
    xa1 = pltpu.make_async_copy(ax.at[pl.ds(X0, M - X0)], x_buf.at[0, pl.ds(X0, M - X0)], sem.at[SEM_XA1])
    xb = pltpu.make_async_copy(bx, x_buf.at[1], sem.at[SEM_XB])

    def wa1(j):
        cols = pl.ds(pl.multiple_of((Q0 + j * Q1) * DH, DH), Q1 * DH)
        return pltpu.make_async_copy(awq.at[:, cols], wq1_buf.at[j], sem.at[SEM_WA1 + j])

    def out_copy(s, b):
        rows = pl.ds(b * SQ, SQ)
        return pltpu.make_async_copy(obuf.at[s, rows], out_hbm.at[rows, pl.ds(s * D, D)], sem.at[SEM_OUT + s * B + b])

    def out_copy_last(j):
        rows, cols = pl.ds((B - 1) * SQ, SQ), pl.ds(j * DH, DH)
        return pltpu.make_async_copy(obuf.at[1, rows, cols], out_hbm.at[rows, pl.ds(D + j * DH, DH)], sem.at[SEM_LAST + j])

    def project(s, w_ref, h0, nh, r0=0, nr=M, c0=0):
        x = x_buf[s, pl.ds(r0, nr), :]
        for t in range(nh):
            q = jnp.dot(x, w_ref[:, (c0 + t) * DH:(c0 + t + 1) * DH], preferred_element_type=jnp.float32)
            q_buf[s, h0 + t, pl.ds(r0, nr), :] = (q * Q_SCALE).astype(jnp.bfloat16)

    def attend(s, g):
        r = s * NG + g
        slot = r & (NGRP - 1)
        for c in group_copies(s, g, slot):
            c.wait()

        def qk(i):
            b, h = divmod(i, GH)
            q = q_buf[s, g * GH + h, b * SQ:(b + 1) * SQ, :]
            return jax.lax.dot_general(q, k_buf[slot, b, h], NT_DIMS, preferred_element_type=jnp.float32)

        def softmax(sc):
            m = jnp.max(sc, axis=-1, keepdims=True)
            p = jnp.exp2(sc - m)
            return p.astype(jnp.bfloat16), jnp.sum(p, axis=-1, keepdims=True)

        def pv(i, p, l):
            b, h = divmod(i, GH)
            o = jnp.dot(p, v_buf[slot, b, h], preferred_element_type=jnp.float32)
            rcp = pl.reciprocal(l, approx=True)
            rcp = rcp * (2.0 - l * rcp)
            return (o * rcp).astype(jnp.bfloat16)

        def out_proj(b, heads):
            o = jnp.concatenate(heads, axis=1)
            rows = pl.ds(b * SQ, SQ)
            last_rows = s == 1 and b == B - 1
            for j in range(D // DH):
                cols = pl.ds(j * DH, DH)
                new = acc[s, rows, cols] + jnp.dot(o, wo_buf[slot, :, cols], preferred_element_type=jnp.float32)
                acc[s, rows, cols] = new
                obuf[s, rows, cols] = new.astype(jnp.bfloat16)
                if last_rows:
                    @pl.when(g == NG - 1)
                    def _():
                        out_copy_last(j).start()

            if not last_rows:
                @pl.when(g == NG - 1)
                def _():
                    out_copy(s, b).start()

        if s == 0:
            project(1, wqb_buf.at[slot], g * GH, GH)
        n_units = B * GH
        sc = qk(0)
        heads, pending = [], None
        for i in range(n_units):
            p, l = softmax(sc)
            if i + 1 < n_units:
                sc = qk(i + 1)
            if pending is not None:
                out_proj(*pending)
                pending = None
            heads.append(pv(i, p, l))
            if len(heads) == GH:
                pending, heads = (i // GH, heads), []
            if i == 1:
                start_group(r + PRO)
        out_proj(*pending)

    xa0.start()
    wa0.start()
    wa0b.start()
    xa1.start()
    for j in range(NQ):
        wa1(j).start()
    start_group(0)
    xb.start()
    for r in range(1, PRO):
        start_group(r)

    def zero_acc(b, carry):
        acc[:, pl.ds(pl.multiple_of(b * SQ, SQ), SQ), :] = jnp.zeros((2, SQ, D), jnp.float32)
        return carry

    jax.lax.fori_loop(0, B, zero_acc, 0)

    def project_rest(j, carry):
        wa1(j).wait()
        project(0, wq1_buf.at[j], Q0 + j * Q1, Q1)
        return carry

    def block(s, carry):
        @pl.when(s == 0)
        def _():
            xa0.wait()
            wa0.wait()
            project(0, wq0_buf, 0, Q0 // 2, 0, X0)
            wa0b.wait()
            project(0, wq0_buf, Q0 // 2, Q0 // 2, 0, X0, Q0 // 2)
            xa1.wait()
            project(0, wq0_buf, 0, Q0, X0, M - X0)
            jax.lax.fori_loop(0, NQ, project_rest, 0)
            xb.wait()

        for blk in range(2):
            @pl.when(s == blk)
            def _():
                def region(g, c):
                    attend(blk, g)
                    return c

                jax.lax.fori_loop(0, NG, region, 0)
        return carry

    jax.lax.fori_loop(0, 2, block, 0)
    for s in range(2):
        for b in range(B - s):
            out_copy(s, b).wait()
    for j in range(D // DH):
        out_copy_last(j).wait()


@jax.jit
def pallas_concat_heads__mha_block_cached__mha_block_cached__near_ridge_kernel(
    A_x: jax.Array,
    A_k_cache: jax.Array,
    A_v_cache: jax.Array,
    A_wq: jax.Array,
    A_wo: jax.Array,
    B_x: jax.Array,
    B_k_cache: jax.Array,
    B_v_cache: jax.Array,
    B_wq: jax.Array,
    B_wo: jax.Array,
):
    hbm = pl.BlockSpec(memory_space=pl.ANY)
    bf16 = jnp.bfloat16
    out = pl.pallas_call(
        _kernel,
        out_shape=jax.ShapeDtypeStruct((M, 2 * D), bf16),
        in_specs=[hbm] * 10,
        out_specs=hbm,
        scratch_shapes=[
            pltpu.VMEM((2, M, D), bf16),
            pltpu.VMEM((D, Q0 * DH), bf16),
            pltpu.VMEM((NQ, D, Q1 * DH), bf16),
            pltpu.VMEM((NGRP, D, GD), bf16),
            pltpu.VMEM((2, H, M, DH), bf16),
            pltpu.VMEM((NGRP, B, GH, SK, DH), bf16),
            pltpu.VMEM((NGRP, B, GH, SK, DH), bf16),
            pltpu.VMEM((NGRP, GD, D), bf16),
            pltpu.VMEM((2, M, D), jnp.float32),
            pltpu.VMEM((2, M, D), bf16),
            pltpu.SemaphoreType.DMA((NUM_SEM,)),
        ],
        compiler_params=pltpu.CompilerParams(
            vmem_limit_bytes=110 * 1024 * 1024,
            disable_bounds_checks=True,
            disable_semaphore_checks=True,
        ),
    )(A_x.reshape(M, D), A_k_cache, A_v_cache, A_wq, A_wo,
      B_x.reshape(M, D), B_k_cache, B_v_cache, B_wq, B_wo)
    return out.reshape(B, SQ, 2 * D)
```

```python
import jax
import jax.numpy as jnp
import jax.experimental.pallas as pl
import jax.experimental.pallas.tpu as pltpu

B, SQ, D, H, SK, DH = 8, 160, 512, 32, 512, 128
M = B * SQ
GH = 4
GD = GH * DH
NG = H // GH
NGRP = 4
PRO = 3
X0 = 480
Q0 = 6
QA = 2
NQ = 2
Q1 = (H - Q0) // NQ
NT_DIMS = (((1,), (1,)), ((), ()))
Q_SCALE = DH ** -0.5 * 1.4426950408889634

SEM_XA0 = NGRP
SEM_XA1 = SEM_XA0 + 1
SEM_WA1 = SEM_XA1 + 1
SEM_XB = SEM_WA1 + NQ
SEM_OUT = SEM_XB + 1
SEM_LAST = SEM_OUT + 2 * B
SEM_WA0B = SEM_LAST + D // DH
NUM_SEM = SEM_WA0B + 1


def _kernel(ax, ak, av, awq, awo, bx, bk, bv, bwq, bwo, out_hbm,
            x_buf, wq0_buf, wq1_buf, wqb_buf, q_buf, k_buf, v_buf, wo_buf, acc, obuf, sem):
    def group_copies(s, g, slot):
        k_hbm, v_hbm, wo_hbm = (ak, av, awo) if s == 0 else (bk, bv, bwo)
        cols = pl.ds(pl.multiple_of(g * GD, GD), GD)
        heads = pl.ds(g * GH, GH)
        copies = [
            pltpu.make_async_copy(k_hbm.at[:, heads], k_buf.at[slot], sem.at[slot]),
            pltpu.make_async_copy(v_hbm.at[:, heads], v_buf.at[slot], sem.at[slot]),
            pltpu.make_async_copy(wo_hbm.at[cols, :], wo_buf.at[slot], sem.at[slot]),
        ]
        if s == 0:
            copies.append(pltpu.make_async_copy(bwq.at[:, cols], wqb_buf.at[slot], sem.at[slot]))
        return copies

    def start_group(r):
        slot, g = r & (NGRP - 1), r & (NG - 1)
        if isinstance(r, int):
            for c in group_copies(r // NG, g, slot):
                c.start()
            return
        for s in range(2):
            @pl.when(jnp.logical_and(r >= s * NG, r < (s + 1) * NG))
            def _():
                for c in group_copies(s, g, slot):
                    c.start()

    xa0 = pltpu.make_async_copy(ax.at[pl.ds(0, X0)], x_buf.at[0, pl.ds(0, X0)], sem.at[SEM_XA0])
    hq = QA * DH
    wa0 = pltpu.make_async_copy(awq.at[:, pl.ds(0, hq)], wq0_buf.at[:, pl.ds(0, hq)], sem.at[SEM_XA0])
    wa0b = pltpu.make_async_copy(awq.at[:, pl.ds(hq, Q0 * DH - hq)], wq0_buf.at[:, pl.ds(hq, Q0 * DH - hq)], sem.at[SEM_WA0B])
    xa1 = pltpu.make_async_copy(ax.at[pl.ds(X0, M - X0)], x_buf.at[0, pl.ds(X0, M - X0)], sem.at[SEM_XA1])
    xb = pltpu.make_async_copy(bx, x_buf.at[1], sem.at[SEM_XB])

    def wa1(j):
        cols = pl.ds(pl.multiple_of((Q0 + j * Q1) * DH, DH), Q1 * DH)
        return pltpu.make_async_copy(awq.at[:, cols], wq1_buf.at[j], sem.at[SEM_WA1 + j])

    def out_copy(s, b):
        rows = pl.ds(b * SQ, SQ)
        return pltpu.make_async_copy(obuf.at[s, rows], out_hbm.at[rows, pl.ds(s * D, D)], sem.at[SEM_OUT + s * B + b])

    def out_copy_last(j):
        rows, cols = pl.ds((B - 1) * SQ, SQ), pl.ds(j * DH, DH)
        return pltpu.make_async_copy(obuf.at[1, rows, cols], out_hbm.at[rows, pl.ds(D + j * DH, DH)], sem.at[SEM_LAST + j])

    def project(s, w_ref, h0, nh, r0=0, nr=M, c0=0):
        x = x_buf[s, pl.ds(r0, nr), :]
        for t in range(nh):
            q = jnp.dot(x, w_ref[:, (c0 + t) * DH:(c0 + t + 1) * DH], preferred_element_type=jnp.float32)
            q_buf[s, h0 + t, pl.ds(r0, nr), :] = (q * Q_SCALE).astype(jnp.bfloat16)

    def attend(s, g):
        r = s * NG + g
        slot = r & (NGRP - 1)
        for c in group_copies(s, g, slot):
            c.wait()

        def qk(i):
            b, h = divmod(i, GH)
            q = q_buf[s, g * GH + h, b * SQ:(b + 1) * SQ, :]
            return jax.lax.dot_general(q, k_buf[slot, b, h], NT_DIMS, preferred_element_type=jnp.float32)

        def softmax(sc):
            m = jnp.max(sc, axis=-1, keepdims=True)
            p = jnp.exp2(sc - m)
            return p.astype(jnp.bfloat16), jnp.sum(p, axis=-1, keepdims=True)

        def pv(i, p, l):
            b, h = divmod(i, GH)
            o = jnp.dot(p, v_buf[slot, b, h], preferred_element_type=jnp.float32)
            rcp = pl.reciprocal(l, approx=True)
            rcp = rcp * (2.0 - l * rcp)
            return (o * rcp).astype(jnp.bfloat16)

        def out_proj(b, heads):
            o = jnp.concatenate(heads, axis=1)
            rows = pl.ds(b * SQ, SQ)
            last_rows = s == 1 and b == B - 1
            for j in range(D // DH):
                cols = pl.ds(j * DH, DH)
                new = acc[s, rows, cols] + jnp.dot(o, wo_buf[slot, :, cols], preferred_element_type=jnp.float32)
                acc[s, rows, cols] = new
                obuf[s, rows, cols] = new.astype(jnp.bfloat16)
                if last_rows:
                    @pl.when(g == NG - 1)
                    def _():
                        out_copy_last(j).start()

            if not last_rows:
                @pl.when(g == NG - 1)
                def _():
                    out_copy(s, b).start()

        if s == 0:
            project(1, wqb_buf.at[slot], g * GH, GH)
        n_units = B * GH
        sc = qk(0)
        heads, pending = [], None
        for i in range(n_units):
            p, l = softmax(sc)
            if i + 1 < n_units:
                sc = qk(i + 1)
            if pending is not None:
                out_proj(*pending)
                pending = None
            heads.append(pv(i, p, l))
            if len(heads) == GH:
                pending, heads = (i // GH, heads), []
            if i == 1:
                start_group(r + PRO)
        out_proj(*pending)

    xa0.start()
    wa0.start()
    wa0b.start()
    xa1.start()
    for j in range(NQ):
        wa1(j).start()
    start_group(0)
    xb.start()
    for r in range(1, PRO):
        start_group(r)

    def zero_acc(b, carry):
        acc[:, pl.ds(pl.multiple_of(b * SQ, SQ), SQ), :] = jnp.zeros((2, SQ, D), jnp.float32)
        return carry

    jax.lax.fori_loop(0, B, zero_acc, 0)

    def project_rest(j, carry):
        wa1(j).wait()
        project(0, wq1_buf.at[j], Q0 + j * Q1, Q1)
        return carry

    def block(s, carry):
        @pl.when(s == 0)
        def _():
            xa0.wait()
            wa0.wait()
            project(0, wq0_buf, 0, QA, 0, X0)
            wa0b.wait()
            project(0, wq0_buf, QA, Q0 - QA, 0, X0, QA)
            xa1.wait()
            project(0, wq0_buf, 0, Q0, X0, M - X0)
            jax.lax.fori_loop(0, NQ, project_rest, 0)
            xb.wait()

        for blk in range(2):
            @pl.when(s == blk)
            def _():
                def region(g, c):
                    attend(blk, g)
                    return c

                jax.lax.fori_loop(0, NG, region, 0)
        return carry

    jax.lax.fori_loop(0, 2, block, 0)
    for s in range(2):
        for b in range(B - s):
            out_copy(s, b).wait()
    for j in range(D // DH):
        out_copy_last(j).wait()


@jax.jit
def pallas_concat_heads__mha_block_cached__mha_block_cached__near_ridge_kernel(
    A_x: jax.Array,
    A_k_cache: jax.Array,
    A_v_cache: jax.Array,
    A_wq: jax.Array,
    A_wo: jax.Array,
    B_x: jax.Array,
    B_k_cache: jax.Array,
    B_v_cache: jax.Array,
    B_wq: jax.Array,
    B_wo: jax.Array,
):
    hbm = pl.BlockSpec(memory_space=pl.ANY)
    bf16 = jnp.bfloat16
    out = pl.pallas_call(
        _kernel,
        out_shape=jax.ShapeDtypeStruct((M, 2 * D), bf16),
        in_specs=[hbm] * 10,
        out_specs=hbm,
        scratch_shapes=[
            pltpu.VMEM((2, M, D), bf16),
            pltpu.VMEM((D, Q0 * DH), bf16),
            pltpu.VMEM((NQ, D, Q1 * DH), bf16),
            pltpu.VMEM((NGRP, D, GD), bf16),
            pltpu.VMEM((2, H, M, DH), bf16),
            pltpu.VMEM((NGRP, B, GH, SK, DH), bf16),
            pltpu.VMEM((NGRP, B, GH, SK, DH), bf16),
            pltpu.VMEM((NGRP, GD, D), bf16),
            pltpu.VMEM((2, M, D), jnp.float32),
            pltpu.VMEM((2, M, D), bf16),
            pltpu.SemaphoreType.DMA((NUM_SEM,)),
        ],
        compiler_params=pltpu.CompilerParams(
            vmem_limit_bytes=110 * 1024 * 1024,
            disable_bounds_checks=True,
            disable_semaphore_checks=True,
        ),
    )(A_x.reshape(M, D), A_k_cache, A_v_cache, A_wq, A_wo,
      B_x.reshape(M, D), B_k_cache, B_v_cache, B_wq, B_wo)
    return out.reshape(B, SQ, 2 * D)
```

```python
import jax
import jax.numpy as jnp
import jax.experimental.pallas as pl
import jax.experimental.pallas.tpu as pltpu

B, SQ, D, H, SK, DH = 8, 160, 512, 32, 512, 128
M = B * SQ
GH = 4
GD = GH * DH
NG = H // GH
NGRP = 4
PRO = 3
X0 = 480
Q0 = 6
QA = 2
NQ = 2
Q1 = (H - Q0) // NQ
QB_AT = (14, 22, 31)
NT_DIMS = (((1,), (1,)), ((), ()))
Q_SCALE = DH ** -0.5 * 1.4426950408889634

SEM_XA0 = NGRP
SEM_XA1 = SEM_XA0 + 1
SEM_WA0B = SEM_XA1 + 1
SEM_WA1 = SEM_WA0B + 1
SEM_XB = SEM_WA1 + NQ
SEM_OUT = SEM_XB + 1
SEM_LAST = SEM_OUT + 2 * B
NUM_SEM = SEM_LAST + D // DH


def _kernel(ax, ak, av, awq, awo, bx, bk, bv, bwq, bwo, out_hbm,
            x_buf, wq0_buf, wq1_buf, wqb_buf, q_buf, k_buf, v_buf, wob_buf, woa_buf, oa_buf,
            acc, obuf, sem):
    def group_copies(s, g, slot):
        k_hbm, v_hbm, wo_hbm = (ak, av, awo) if s == 0 else (bk, bv, bwo)
        cols = pl.ds(pl.multiple_of(g * GD, GD), GD)
        heads = pl.ds(g * GH, GH)
        copies = [
            pltpu.make_async_copy(k_hbm.at[:, heads], k_buf.at[slot], sem.at[slot]),
            pltpu.make_async_copy(v_hbm.at[:, heads], v_buf.at[slot], sem.at[slot]),
            pltpu.make_async_copy(wo_hbm.at[cols, :], woa_buf.at[g] if s == 0 else wob_buf.at[slot], sem.at[slot]),
        ]
        if s == 0:
            copies.append(pltpu.make_async_copy(bwq.at[:, cols], wqb_buf.at[slot], sem.at[slot]))
        return copies

    def start_group(r):
        slot, g = r & (NGRP - 1), r & (NG - 1)
        if isinstance(r, int):
            for c in group_copies(r // NG, g, slot):
                c.start()
            return
        for s in range(2):
            @pl.when(jnp.logical_and(r >= s * NG, r < (s + 1) * NG))
            def _():
                for c in group_copies(s, g, slot):
                    c.start()

    wq_a = QA * DH
    wq_b = Q0 * DH - wq_a
    xa0 = pltpu.make_async_copy(ax.at[pl.ds(0, X0)], x_buf.at[0, pl.ds(0, X0)], sem.at[SEM_XA0])
    wa0 = pltpu.make_async_copy(awq.at[:, pl.ds(0, wq_a)], wq0_buf.at[:, pl.ds(0, wq_a)], sem.at[SEM_XA0])
    wa0b = pltpu.make_async_copy(awq.at[:, pl.ds(wq_a, wq_b)], wq0_buf.at[:, pl.ds(wq_a, wq_b)], sem.at[SEM_WA0B])
    xa1 = pltpu.make_async_copy(ax.at[pl.ds(X0, M - X0)], x_buf.at[0, pl.ds(X0, M - X0)], sem.at[SEM_XA1])
    xb = pltpu.make_async_copy(bx, x_buf.at[1], sem.at[SEM_XB])

    def wa1(j):
        cols = pl.ds(pl.multiple_of((Q0 + j * Q1) * DH, DH), Q1 * DH)
        return pltpu.make_async_copy(awq.at[:, cols], wq1_buf.at[j], sem.at[SEM_WA1 + j])

    def out_copy(s, b):
        rows = pl.ds(b * SQ, SQ)
        return pltpu.make_async_copy(obuf.at[s, rows], out_hbm.at[rows, pl.ds(s * D, D)], sem.at[SEM_OUT + s * B + b])

    def out_copy_last(j):
        rows, cols = pl.ds((B - 1) * SQ, SQ), pl.ds(j * DH, DH)
        return pltpu.make_async_copy(obuf.at[1, rows, cols], out_hbm.at[rows, pl.ds(D + j * DH, DH)], sem.at[SEM_LAST + j])

    def project(s, w_ref, c0, h0, nh, r0=0, nr=M):
        x = x_buf[s, pl.ds(r0, nr), :]
        for t in range(nh):
            q = jnp.dot(x, w_ref[:, (c0 + t) * DH:(c0 + t + 1) * DH], preferred_element_type=jnp.float32)
            q_buf[s, h0 + t, pl.ds(r0, nr), :] = (q * Q_SCALE).astype(jnp.bfloat16)

    def attend(s, g):
        slot = (s * NG + g) & (NGRP - 1)
        for c in group_copies(s, g, slot):
            c.wait()

        def qk(i):
            b, h = divmod(i, GH)
            q = q_buf[s, g * GH + h, b * SQ:(b + 1) * SQ, :]
            return jax.lax.dot_general(q, k_buf[slot, b, h], NT_DIMS, preferred_element_type=jnp.float32)

        def softmax(sc):
            m = jnp.max(sc, axis=-1, keepdims=True)
            p = jnp.exp2(sc - m)
            return p.astype(jnp.bfloat16), jnp.sum(p, axis=-1, keepdims=True)

        def pv(i, p, l):
            b, h = divmod(i, GH)
            o = jnp.dot(p, v_buf[slot, b, h], preferred_element_type=jnp.float32)
            rcp = pl.reciprocal(l, approx=True)
            rcp = rcp * (2.0 - l * rcp)
            return (o * rcp).astype(jnp.bfloat16)

        def out_proj(t, b, o):
            rows = pl.ds(b * SQ, SQ)
            w = woa_buf.at[g] if t == 0 else wob_buf.at[slot]
            last_rows = t == 1 and b == B - 1
            for j in range(D // DH):
                cols = pl.ds(j * DH, DH)
                new = acc[t, rows, cols] + jnp.dot(o, w[:, cols], preferred_element_type=jnp.float32)
                acc[t, rows, cols] = new
                obuf[t, rows, cols] = new.astype(jnp.bfloat16)
                if last_rows:
                    @pl.when(g == NG - 1)
                    def _():
                        out_copy_last(j).start()

            if not last_rows:
                @pl.when(g == NG - 1)
                def _():
                    out_copy(t, b).start()

        if s == 0:
            project(1, wqb_buf.at[slot], 0, g * GH, 1)
        else:
            out_proj(0, B - 1, oa_buf[g])
        n_units = B * GH
        sc = qk(0)
        heads, pending = [], None
        for i in range(n_units):
            p, l = softmax(sc)
            if i + 1 < n_units:
                sc = qk(i + 1)
            if pending is not None:
                out_proj(s, *pending)
                pending = None
            heads.append(pv(i, p, l))
            if s == 0 and i in QB_AT:
                t = 1 + QB_AT.index(i)
                project(1, wqb_buf.at[slot], t, g * GH + t, 1)
            if len(heads) == GH:
                pending, heads = (i // GH, jnp.concatenate(heads, axis=1)), []
            if i == 5:
                start_group(s * NG + g + PRO)
        if s == 0:
            oa_buf[g] = pending[1]
        else:
            out_proj(s, *pending)

    xa0.start()
    wa0.start()
    wa0b.start()
    xa1.start()
    for j in range(NQ):
        wa1(j).start()
    start_group(0)
    xb.start()
    for r in range(1, PRO):
        start_group(r)

    def zero_acc(b, carry):
        acc[:, pl.ds(pl.multiple_of(b * SQ, SQ), SQ), :] = jnp.zeros((2, SQ, D), jnp.float32)
        return carry

    def project_rest(j, carry):
        wa1(j).wait()
        project(0, wq1_buf.at[j], 0, Q0 + j * Q1, Q1)
        return carry

    def block(s, carry):
        @pl.when(s == 0)
        def _():
            jax.lax.fori_loop(0, B, zero_acc, 0)
            xa0.wait()
            wa0.wait()
            project(0, wq0_buf, 0, 0, QA, 0, X0)
            wa0b.wait()
            project(0, wq0_buf, QA, QA, Q0 - QA, 0, X0)
            xa1.wait()
            project(0, wq0_buf, 0, 0, Q0, X0, M - X0)
            jax.lax.fori_loop(0, NQ, project_rest, 0)
            xb.wait()

        for blk in range(2):
            @pl.when(s == blk)
            def _():
                def region(g, c):
                    attend(blk, g)
                    return c

                jax.lax.fori_loop(0, NG, region, 0)
        return carry

    jax.lax.fori_loop(0, 2, block, 0)
    for s in range(2):
        for b in range(B - s):
            out_copy(s, b).wait()
    for j in range(D // DH):
        out_copy_last(j).wait()


@jax.jit
def pallas_concat_heads__mha_block_cached__mha_block_cached__near_ridge_kernel(
    A_x: jax.Array,
    A_k_cache: jax.Array,
    A_v_cache: jax.Array,
    A_wq: jax.Array,
    A_wo: jax.Array,
    B_x: jax.Array,
    B_k_cache: jax.Array,
    B_v_cache: jax.Array,
    B_wq: jax.Array,
    B_wo: jax.Array,
):
    hbm = pl.BlockSpec(memory_space=pl.ANY)
    bf16 = jnp.bfloat16
    out = pl.pallas_call(
        _kernel,
        out_shape=jax.ShapeDtypeStruct((M, 2 * D), bf16),
        in_specs=[hbm] * 10,
        out_specs=hbm,
        scratch_shapes=[
            pltpu.VMEM((2, M, D), bf16),
            pltpu.VMEM((D, Q0 * DH), bf16),
            pltpu.VMEM((NQ, D, Q1 * DH), bf16),
            pltpu.VMEM((NGRP, D, GD), bf16),
            pltpu.VMEM((2, H, M, DH), bf16),
            pltpu.VMEM((NGRP, B, GH, SK, DH), bf16),
            pltpu.VMEM((NGRP, B, GH, SK, DH), bf16),
            pltpu.VMEM((NGRP, GD, D), bf16),
            pltpu.VMEM((NG, GD, D), bf16),
            pltpu.VMEM((NG, SQ, GD), bf16),
            pltpu.VMEM((2, M, D), jnp.float32),
            pltpu.VMEM((2, M, D), bf16),
            pltpu.SemaphoreType.DMA((NUM_SEM,)),
        ],
        compiler_params=pltpu.CompilerParams(
            vmem_limit_bytes=110 * 1024 * 1024,
            disable_bounds_checks=True,
            disable_semaphore_checks=True,
        ),
    )(A_x.reshape(M, D), A_k_cache, A_v_cache, A_wq, A_wo,
      B_x.reshape(M, D), B_k_cache, B_v_cache, B_wq, B_wo)
    return out.reshape(B, SQ, 2 * D)
```
